```python
import os as _os
_os.environ.setdefault('JAX_PLATFORMS', 'cpu')
import jax
import jax.numpy as jnp

def _softmax(x, axis=-1):
    return jax.nn.softmax(x, axis=axis)

def _gelu(x):
    return jax.nn.gelu(x, approximate=True)

def _silu(x):
    return jax.nn.silu(x)

def _sigmoid(x):
    return jax.nn.sigmoid(x)

def _layernorm(x, axis=-1, eps=1e-05):
    m = jnp.mean(x, axis=axis, keepdims=True)
    v = jnp.var(x, axis=axis, keepdims=True)
    return (x - m) / jnp.sqrt(v + eps)

def _scatter_add(tgt, idx, src, axis=0):
    return tgt.at[idx].add(src)

def _segment_sum(src, seg, n):
    return jax.ops.segment_sum(src, seg, n)

class _Rng:

    def __init__(self, key):
        self._k = key

    def _next(self):
        self._k, sub = jax.random.split(self._k)
        return sub

    def normal(self, shape):
        return jax.random.normal(self._next(), shape, dtype=jnp.bfloat16)

    def randint(self, lo, hi, shape):
        return jax.random.randint(self._next(), shape, lo, hi, dtype=jnp.int32)

    def uniform(self, shape, lo=0.0, hi=1.0):
        return jax.random.uniform(self._next(), shape, jnp.bfloat16, lo, hi)

    def permutation(self, n):
        return jax.random.permutation(self._next(), n)
kernel_name = 'standalone__conformer_conv_module__speech'

def setup_inputs():
    _rng = _Rng(jax.random.key(int.from_bytes(__import__("os").urandom(4), "little")))
    _w = lambda a: (lambda t: t.astype(jnp.bfloat16) if jnp.issubdtype(t.dtype, jnp.floating) else t)(jnp.asarray(a))
    B, T, D, K = (2, 16000, 256, 5)
    return {'x': _w((lambda *s: _rng.normal(s) * 0.2)(B, T, D)), 'w_pw1': _w((lambda *s: _rng.normal(s) * 0.2)(D, 2 * D)), 'dw': _w((lambda *s: _rng.normal(s) * 0.05)(K, D)), 'w_pw2': _w((lambda *s: _rng.normal(s) * 0.05)(D, D))}

def reference(x, w_pw1, dw, w_pw2):
    B, T, D = x.shape
    K = dw.shape[0]
    h = x @ w_pw1
    a, b = (h[..., :D].copy(), h[..., D:].copy())
    h = a * _sigmoid(b)
    pad = K // 2
    hp = jnp.pad(h, ((0, 0), (pad, pad), (0, 0)))
    out = jnp.zeros_like(h)
    for i in range(K):
        out = out + hp[:, i:i + T, :] * dw[i][None, None, :]
    return _silu(out) @ w_pw2
```

```python
import jax
import jax.numpy as jnp
from jax import lax
import jax.experimental.pallas as pl
import jax.experimental.pallas.tpu as pltpu

LANES = 128
HALO = 16
CHUNK = 400
DIST = 3
NSEM = 10


def _pick_chunk(t):
    for m in (CHUNK, 512, 384, 320, 256, 192, 128, 64, 32):
        if t % m == 0:
            return m
    raise ValueError("sequence length must be a multiple of 32")


@jax.jit
def pallas_standalone__conformer_conv_module__speech_kernel(
    x: jax.Array,
    w_pw1: jax.Array,
    dw: jax.Array,
    w_pw2: jax.Array,
):
    B, T, D = x.shape
    K = dw.shape[0]
    P = K // 2
    L, H = LANES, HALO
    N = B * T
    M = _pick_chunk(T)
    U = T // M
    R = T
    n_ch = N // M
    NC = D // L
    dist = DIST
    S = NSEM if U % NSEM == 0 else U
    assert D % L == 0 and D % 16 == 0 and P <= 8 and dist <= S and U >= 2

    def kernel_function(x_hbm, w1_hbm, dw_hbm, w2_hbm, o_hbm,
                        x_v, xp_v, o_v, h_v, w1_v, dw_v, w2_v, w1s, dws,
                        in_sems, w_sems, out_sem):
        def x_copy(j, sem_idx):
            src = jnp.minimum(j * M + H, N - M)
            return pltpu.make_async_copy(
                x_hbm.at[pl.ds(pl.multiple_of(src, H), M), :],
                x_v.at[pl.ds(pl.multiple_of(j * M, M), M), :],
                in_sems.at[sem_idx])

        def o_copy(r0):
            rows = pl.ds(pl.multiple_of(r0, M), M)
            return pltpu.make_async_copy(o_v.at[rows, :], o_hbm.at[rows, :], out_sem.at[0])

        cw1 = pltpu.make_async_copy(w1_hbm, w1_v, w_sems.at[0])
        cdw = pltpu.make_async_copy(dw_hbm, dw_v, w_sems.at[1])
        cw2 = pltpu.make_async_copy(w2_hbm, w2_v, w_sems.at[2])
        cxp = pltpu.make_async_copy(x_hbm.at[pl.ds(0, H), :], xp_v, w_sems.at[3])

        def issue(j, carry):
            @pl.when(j == 0)
            def _():
                cw1.start()
                cxp.start()
                cdw.start()
            x_copy(j, j % S).start()

            @pl.when(j == 0)
            def _():
                cw2.start()
            return carry
        lax.fori_loop(0, dist, issue, 0)

        cw1.wait()
        for c in range(NC):
            wa = w1_v[:, c * L:(c + 1) * L].astype(jnp.float32) * 0.5
            wb = w1_v[:, D + c * L:D + (c + 1) * L].astype(jnp.float32) * 0.5
            wc = jnp.concatenate([wa, wb], axis=1).astype(jnp.bfloat16)
            w1s[c] = pltpu.bitcast(wc, jnp.uint32)
        cdw.wait()
        dwv = dw_v[...].astype(jnp.float32) * 0.5
        for i in range(K):
            for c in range(NC):
                dws[i, c] = jnp.broadcast_to(dwv[i:i + 1, c * L:(c + 1) * L], (8, L))

        def w1_tile(c):
            return pltpu.bitcast(w1s[c], jnp.bfloat16)

        def glu(hh):
            a = hh[:, :L]
            return a + a * jnp.tanh(hh[:, L:])

        cxp.wait()
        x0 = xp_v[...]
        for c in range(NC):
            h_v[c, pl.ds(H, H), :] = glu(jnp.dot(x0, w1_tile(c), preferred_element_type=jnp.float32))
            h_v[c, pl.ds(0, H), :] = jnp.zeros((H, L), jnp.float32)
        x_copy(0, 0).wait()
        cw2.wait()

        def stage_glu(i, base, u, dma_mid):
            r0 = base + u * M
            if u == U - 1:
                r0 = pl.multiple_of(r0 + jnp.where(i == B - 1, H, 0), H)
            xv = x_v[pl.ds(r0, M), :]
            for c in range(NC):
                hh = jnp.dot(xv, w1_tile(c), preferred_element_type=jnp.float32)
                if c == 0:
                    dma_mid()
                g = glu(hh)
                if u < U - 1:
                    h_v[c, pl.ds(2 * H + u * M, M), :] = g
                else:
                    h_v[c, pl.ds(2 * H + u * M, M - H), :] = g[:M - H]
                    h_v[c, pl.ds(R + H, 8), :] = jnp.zeros((8, L), jnp.float32)
                    h_v[c, pl.ds(H, H), :] = g[M - H:]
                    h_v[c, pl.ds(H - 8, 8), :] = jnp.zeros((8, L), jnp.float32)

        def stage_conv_out(base, u):
            ys = []
            for c in range(NC):
                acc = None
                for k in range(K):
                    w = jnp.tile(dws[k, c], (M // 8, 1))
                    t = h_v[c, pl.ds(H + u * M - P + k, M), :] * w
                    acc = t if acc is None else acc + t
                ys.append(acc + acc * jnp.tanh(acc))
            y = jnp.concatenate(ys, axis=1).astype(jnp.bfloat16)
            o = jnp.dot(y, w2_v[...], preferred_element_type=jnp.float32)
            o_v[pl.ds(base + u * M, M), :] = o.astype(o_v.dtype)

        def batch_step(i, carry):
            base = pl.multiple_of(i * R, R)
            for u in range(U):
                c = i * U + u

                def dma_mid(u=u, c=c):
                    if u > 0:
                        o_copy(base + (u - 1) * M).start()
                    if u < U - 1:
                        x_copy(c + 1, (u + 1) % S).wait()
                    if u == U - 2:
                        x_copy(c + 2, (u + 2) % S).wait()
                    x_copy(c + dist, (u + dist) % S).start()
                stage_glu(i, base, u, dma_mid)
                stage_conv_out(base, u)
            o_copy(base + (U - 1) * M).start()
            return carry
        lax.fori_loop(0, B, batch_step, 0)

        for j in range(n_ch + 1, n_ch + dist):
            x_copy(j, j % S).wait()
        pltpu.make_async_copy(o_v, o_hbm, out_sem.at[0]).wait()

    out = pl.pallas_call(
        kernel_function,
        in_specs=[pl.BlockSpec(memory_space=pl.ANY)] * 4,
        out_specs=pl.BlockSpec(memory_space=pl.ANY),
        out_shape=jax.ShapeDtypeStruct((N, D), x.dtype),
        scratch_shapes=[
            pltpu.VMEM(((n_ch + dist) * M, D), x.dtype),
            pltpu.VMEM((H, D), x.dtype),
            pltpu.VMEM((N, D), x.dtype),
            pltpu.VMEM((NC, R + 2 * H, L), jnp.float32),
            pltpu.VMEM((D, 2 * D), w_pw1.dtype),
            pltpu.VMEM((K, D), dw.dtype),
            pltpu.VMEM((D, D), w_pw2.dtype),
            pltpu.VMEM((NC, D // 2, 2 * L), jnp.uint32),
            pltpu.VMEM((K, NC, 8, L), jnp.float32),
            pltpu.SemaphoreType.DMA((S,)),
            pltpu.SemaphoreType.DMA((4,)),
            pltpu.SemaphoreType.DMA((1,)),
        ],
        compiler_params=pltpu.CompilerParams(
            vmem_limit_bytes=100 * 1024 * 1024,
            disable_bounds_checks=True,
            disable_semaphore_checks=True,
            flags={"XLA_TPU_RESCHEDULE_DMA_DONES": True},
        ),
    )(x.reshape(N, D), w_pw1, dw, w_pw2)
    return out.reshape(B, T, D)
```

```python
import jax
import jax.numpy as jnp
from jax import lax
import jax.experimental.pallas as pl
import jax.experimental.pallas.tpu as pltpu

LANES = 128
HALO = 16
CHUNK = 400
DIST = 3


def _plan(t):
    for m in (CHUNK, 512, 384, 320, 256, 192, 160, 128, 96):
        if t % m == 0 and t // m > DIST:
            break
    else:
        raise ValueError("unsupported sequence length: %d" % t)
    first = (2 * m // 5) // HALO * HALO
    sizes = [first, m - first] + [m] * (t // m - 1)
    piece = max((m // 5) // HALO * HALO, HALO)
    pieces = [piece] * (m // piece)
    pieces[0] += m - sum(pieces)
    return sizes, pieces


@jax.jit
def pallas_standalone__conformer_conv_module__speech_kernel(
    x: jax.Array,
    w_pw1: jax.Array,
    dw: jax.Array,
    w_pw2: jax.Array,
):
    B, T, D = x.shape
    K = dw.shape[0]
    P = K // 2
    L, H = LANES, HALO
    N = B * T
    NC = D // L
    assert D % L == 0 and P <= 8 and T % H == 0

    sizes, tail_pieces = _plan(T)
    U = len(sizes)
    offs = [sum(sizes[:u]) for u in range(U + 1)]
    ga = [0 if u == 0 else offs[u] + H for u in range(U)]
    gb = [min(offs[u + 1] + H, T) for u in range(U)]

    schedule, nxt = [], 0
    for u in range(U):
        upto = u + 1 if u + 1 < U - 1 else u
        while nxt <= upto:
            schedule.append(("glu", nxt))
            nxt += 1
        schedule.append(("out", u))

    def kernel_function(x_hbm, w1_hbm, dw_hbm, w2_hbm, o_hbm,
                        x_v, o_v, h_v, w1_v, dw_v, w2_v, w1s, dws,
                        in_sems, w_sems, out_sem):
        def x_copy(i, u):
            i, u = i + u // U, u % U
            n = gb[u] - ga[u]
            return pltpu.make_async_copy(
                x_hbm.at[pl.ds(pl.multiple_of(i * T + ga[u], H), n), :],
                x_v.at[i % 2, pl.ds(ga[u], n), :],
                in_sems.at[u])

        def o_copy(row0, n):
            rows = pl.ds(pl.multiple_of(row0, H), n)
            return pltpu.make_async_copy(o_v.at[rows, :], o_hbm.at[rows, :], out_sem.at[0])

        cw1 = pltpu.make_async_copy(w1_hbm, w1_v, w_sems.at[0])
        cdw = pltpu.make_async_copy(dw_hbm, dw_v, w_sems.at[1])
        cw2 = pltpu.make_async_copy(w2_hbm, w2_v, w_sems.at[2])

        def issue(i, carry):
            cw1.start()
            cdw.start()
            x_copy(i, 0).start()
            cw2.start()
            for q in range(1, DIST):
                x_copy(i, q).start()
            return carry
        lax.fori_loop(0, pl.program_id(0) + 1, issue, 0)

        cw1.wait()
        for c in range(NC):
            wa = w1_v[:, c * L:(c + 1) * L].astype(jnp.float32) * 0.5
            wb = w1_v[:, D + c * L:D + (c + 1) * L].astype(jnp.float32) * 0.5
            wc = jnp.concatenate([wa, wb], axis=1).astype(w1_v.dtype)
            w1s[c] = pltpu.bitcast(wc, jnp.uint32)
        cdw.wait()
        dwv = dw_v[...].astype(jnp.float32) * 0.5
        for k in range(K):
            for c in range(NC):
                dws[k, c] = jnp.broadcast_to(dwv[k:k + 1, c * L:(c + 1) * L], (8, L))
        for c in range(NC):
            h_v[c, pl.ds(0, H), :] = jnp.zeros((H, L), jnp.float32)
            h_v[c, pl.ds(H + T, 8), :] = jnp.zeros((8, L), jnp.float32)

        def stage_glu(i, u):
            if u + DIST < U:
                x_copy(i, u + DIST).start()
            else:
                @pl.when(i + 1 < B)
                def _():
                    x_copy(i, u + DIST).start()
            x_copy(i, u).wait()
            n = gb[u] - ga[u]
            xv = x_v[i % 2, pl.ds(ga[u], n), :]
            for c in range(NC):
                hh = jnp.dot(xv, pltpu.bitcast(w1s[c], x_v.dtype), preferred_element_type=jnp.float32)
                a = hh[:, :L]
                h_v[c, pl.ds(H + ga[u], n), :] = a + a * jnp.tanh(hh[:, L:])

        def stage_out(i, u):
            m = sizes[u]
            ys = []
            for c in range(NC):
                acc = None
                for k in range(K):
                    w = jnp.tile(dws[k, c], (m // 8, 1))
                    t = h_v[c, pl.ds(H + offs[u] - P + k, m), :] * w
                    acc = t if acc is None else acc + t
                ys.append(acc + acc * jnp.tanh(acc))
            y = jnp.concatenate(ys, axis=1).astype(w2_v.dtype)
            if u == 0:
                @pl.when(i == 0)
                def _():
                    cw2.wait()
            o = jnp.dot(y, w2_v[...], preferred_element_type=jnp.float32).astype(o_v.dtype)
            r = 0
            for n in (tail_pieces if u == U - 1 else [m]):
                row0 = i * T + (offs[u] + r)
                o_v[pl.ds(pl.multiple_of(row0, H), n), :] = o[r:r + n]
                o_copy(row0, n).start()
                r += n

        def batch_step(i, carry):
            for kind, u in schedule:
                (stage_glu if kind == "glu" else stage_out)(i, u)
            return carry
        lax.fori_loop(0, B, batch_step, 0)

        pltpu.make_async_copy(o_v, o_hbm, out_sem.at[0]).wait()

    out = pl.pallas_call(
        kernel_function,
        grid=(1,),
        in_specs=[pl.BlockSpec(memory_space=pl.ANY)] * 4,
        out_specs=pl.BlockSpec(memory_space=pl.ANY),
        out_shape=jax.ShapeDtypeStruct((N, D), x.dtype),
        scratch_shapes=[
            pltpu.VMEM((2, T, D), x.dtype),
            pltpu.VMEM((N, D), x.dtype),
            pltpu.VMEM((NC, T + 2 * H, L), jnp.float32),
            pltpu.VMEM((D, 2 * D), w_pw1.dtype),
            pltpu.VMEM((K, D), dw.dtype),
            pltpu.VMEM((D, D), w_pw2.dtype),
            pltpu.VMEM((NC, D // 2, 2 * L), jnp.uint32),
            pltpu.VMEM((K, NC, 8, L), jnp.float32),
            pltpu.SemaphoreType.DMA((U,)),
            pltpu.SemaphoreType.DMA((3,)),
            pltpu.SemaphoreType.DMA((1,)),
        ],
        compiler_params=pltpu.CompilerParams(
            dimension_semantics=("arbitrary",),
            vmem_limit_bytes=100 * 1024 * 1024,
            disable_bounds_checks=True,
            disable_semaphore_checks=True,
            flags={"XLA_TPU_RESCHEDULE_DMA_DONES": True},
        ),
    )(x.reshape(N, D), w_pw1, dw, w_pw2)
    return out.reshape(B, T, D)
```

```python
import jax
import jax.numpy as jnp
from jax import lax
import jax.experimental.pallas as pl
import jax.experimental.pallas.tpu as pltpu

LANES = 128
HALO = 16
CHUNK = 400
DIST = 3


def _plan(t):
    for m in (CHUNK, 512, 384, 320, 256, 192, 160, 128, 96):
        if t % m == 0 and t // m > DIST:
            break
    else:
        raise ValueError("unsupported sequence length: %d" % t)
    first = (2 * m // 5) // HALO * HALO
    sizes = [first, m - first] + [m] * (t // m - 1)
    piece = max((m // 5) // HALO * HALO, HALO)
    pieces = [piece] * (m // piece)
    pieces[0] += m - sum(pieces)
    return sizes, pieces


@jax.jit
def pallas_standalone__conformer_conv_module__speech_kernel(
    x: jax.Array,
    w_pw1: jax.Array,
    dw: jax.Array,
    w_pw2: jax.Array,
):
    B, T, D = x.shape
    K = dw.shape[0]
    P = K // 2
    L, H = LANES, HALO
    N = B * T
    NC = D // L
    assert D % L == 0 and P <= 8 and T % H == 0

    sizes, tail_pieces = _plan(T)
    U = len(sizes)
    offs = [sum(sizes[:u]) for u in range(U + 1)]
    ga = [0 if u == 0 else offs[u] + H for u in range(U)]
    gb = [min(offs[u + 1] + H, T) for u in range(U)]

    schedule, nxt = [], 0
    for u in range(U):
        upto = u + 1 if u + 1 < U - 1 else u
        while nxt <= upto:
            schedule.append(("glu", nxt))
            nxt += 1
        schedule.append(("out", u))

    def kernel_function(x_hbm, w1_hbm, dw_hbm, w2_hbm, o_hbm,
                        x_v, o_v, h_v, w1_v, dw_v, w2_v, w1s, dws,
                        in_sems, w_sems, out_sems):
        def x_copy(i, u):
            i, u = i + u // U, u % U
            n = gb[u] - ga[u]
            return pltpu.make_async_copy(
                x_hbm.at[pl.ds(pl.multiple_of(i * T + ga[u], H), n), :],
                x_v.at[i % 2, pl.ds(ga[u], n), :],
                in_sems.at[u])

        def o_copy(i, r, n):
            return pltpu.make_async_copy(
                o_v.at[i % 2, pl.ds(r, n), :],
                o_hbm.at[pl.ds(pl.multiple_of(i * T + r, H), n), :],
                out_sems.at[i % 2])

        cw1 = pltpu.make_async_copy(w1_hbm, w1_v, w_sems.at[0])
        cdw = pltpu.make_async_copy(dw_hbm, dw_v, w_sems.at[1])
        cw2 = pltpu.make_async_copy(w2_hbm, w2_v, w_sems.at[2])

        def issue(i, carry):
            cw1.start()
            cdw.start()
            x_copy(i, 0).start()
            cw2.start()
            for q in range(1, DIST):
                x_copy(i, q).start()
            return carry
        lax.fori_loop(0, pl.program_id(0) + 1, issue, 0)

        cw1.wait()
        for c in range(NC):
            wa = w1_v[:, c * L:(c + 1) * L].astype(jnp.float32) * 0.5
            wb = w1_v[:, D + c * L:D + (c + 1) * L].astype(jnp.float32) * 0.5
            wc = jnp.concatenate([wa, wb], axis=1).astype(w1_v.dtype)
            w1s[c] = pltpu.bitcast(wc, jnp.uint32)
        cdw.wait()
        dwv = dw_v[...].astype(jnp.float32) * 0.5
        for k in range(K):
            for c in range(NC):
                dws[k, c] = jnp.broadcast_to(dwv[k:k + 1, c * L:(c + 1) * L], (8, L))
        for c in range(NC):
            h_v[c, pl.ds(0, H), :] = jnp.zeros((H, L), jnp.float32)
            h_v[c, pl.ds(H + T, 8), :] = jnp.zeros((8, L), jnp.float32)

        def stage_glu(i, u):
            if u + DIST < U:
                x_copy(i, u + DIST).start()
            else:
                @pl.when(i + 1 < B)
                def _():
                    x_copy(i, u + DIST).start()
            x_copy(i, u).wait()
            n = gb[u] - ga[u]
            xv = x_v[i % 2, pl.ds(ga[u], n), :]
            for c in range(NC):
                hh = jnp.dot(xv, pltpu.bitcast(w1s[c], x_v.dtype), preferred_element_type=jnp.float32)
                a = hh[:, :L]
                h_v[c, pl.ds(H + ga[u], n), :] = a + a * jnp.tanh(hh[:, L:])

        def stage_out(i, u):
            m = sizes[u]
            ys = []
            for c in range(NC):
                acc = None
                for k in range(K):
                    w = jnp.tile(dws[k, c], (m // 8, 1))
                    t = h_v[c, pl.ds(H + offs[u] - P + k, m), :] * w
                    acc = t if acc is None else acc + t
                ys.append(acc + acc * jnp.tanh(acc))
            y = jnp.concatenate(ys, axis=1).astype(w2_v.dtype)
            if u == 0:
                @pl.when(i == 0)
                def _():
                    cw2.wait()
            o = jnp.dot(y, w2_v[...], preferred_element_type=jnp.float32).astype(o_v.dtype)
            r = 0
            for n in (tail_pieces if u == U - 1 else [m]):
                o_v[i % 2, pl.ds(offs[u] + r, n), :] = o[r:r + n]
                o_copy(i, offs[u] + r, n).start()
                r += n

        def batch_step(i, carry):
            @pl.when(i >= 2)
            def _():
                o_copy(i - 2, 0, T).wait()
            for kind, u in schedule:
                (stage_glu if kind == "glu" else stage_out)(i, u)
            return carry
        lax.fori_loop(0, B, batch_step, 0)

        for i in range(max(B - 2, 0), B):
            o_copy(i, 0, T).wait()

    out = pl.pallas_call(
        kernel_function,
        grid=(1,),
        in_specs=[pl.BlockSpec(memory_space=pl.ANY)] * 4,
        out_specs=pl.BlockSpec(memory_space=pl.ANY),
        out_shape=jax.ShapeDtypeStruct((N, D), x.dtype),
        scratch_shapes=[
            pltpu.VMEM((2, T, D), x.dtype),
            pltpu.VMEM((2, T, D), x.dtype),
            pltpu.VMEM((NC, T + 2 * H, L), jnp.float32),
            pltpu.VMEM((D, 2 * D), w_pw1.dtype),
            pltpu.VMEM((K, D), dw.dtype),
            pltpu.VMEM((D, D), w_pw2.dtype),
            pltpu.VMEM((NC, D // 2, 2 * L), jnp.uint32),
            pltpu.VMEM((K, NC, 8, L), jnp.float32),
            pltpu.SemaphoreType.DMA((U,)),
            pltpu.SemaphoreType.DMA((3,)),
            pltpu.SemaphoreType.DMA((2,)),
        ],
        compiler_params=pltpu.CompilerParams(
            dimension_semantics=("arbitrary",),
            vmem_limit_bytes=100 * 1024 * 1024,
            disable_bounds_checks=True,
            disable_semaphore_checks=True,
            flags={"XLA_TPU_RESCHEDULE_DMA_DONES": True},
        ),
    )(x.reshape(N, D), w_pw1, dw, w_pw2)
    return out.reshape(B, T, D)
```
